```python
import os as _os
_os.environ.setdefault("JAX_PLATFORMS", "cpu")
import jax
import jax.numpy as jnp

def _softmax(x, axis=-1):
    return jax.nn.softmax(x, axis=axis)
def _gelu(x):
    return jax.nn.gelu(x, approximate=True)
def _silu(x):
    return jax.nn.silu(x)
def _sigmoid(x):
    return jax.nn.sigmoid(x)
def _layernorm(x, axis=-1, eps=1e-5):
    m = jnp.mean(x, axis=axis, keepdims=True)
    v = jnp.var(x, axis=axis, keepdims=True)
    return (x - m) / jnp.sqrt(v + eps)
def _scatter_add(tgt, idx, src, axis=0):
    return tgt.at[idx].add(src)
def _segment_sum(src, seg, n):
    return jax.ops.segment_sum(src, seg, n)
class _Rng:
    def __init__(self, key):
        self._k = key
    def _next(self):
        self._k, sub = jax.random.split(self._k)
        return sub
    def normal(self, shape):
        return jax.random.normal(self._next(), shape, dtype=jnp.bfloat16)
    def randint(self, lo, hi, shape):
        return jax.random.randint(self._next(), shape, lo, hi, dtype=jnp.int32)
    def uniform(self, shape, lo=0.0, hi=1.0):
        return jax.random.uniform(self._next(), shape, jnp.bfloat16, lo, hi)
    def permutation(self, n):
        return jax.random.permutation(self._next(), n)


kernel_name = 'recurrent_scan__spectral_gfnet__swiglu_ffn__prompt'

def setup_inputs():
    _rng = _Rng(jax.random.key(int.from_bytes(__import__("os").urandom(4), "little")))
    _w = (lambda a: (lambda t: t.astype(jnp.bfloat16) if jnp.issubdtype(t.dtype, jnp.floating) else t)(jnp.asarray(a)))
    def _A_setup():
        B, S, D = 1, 2048, 640
        Df = D // 2 + 1
        return {
            "x": _w((lambda *s: _rng.normal(s) * 0.05)(B, S, D)),
            "w_r": _w((lambda *s: _rng.normal(s) * 0.05)(S, Df) * 0.02),
            "w_i": _w((lambda *s: _rng.normal(s) * 0.05)(S, Df) * 0.02),
        }
    _A_in = _A_setup()

    def _B_setup():
        B, S, D, F = 1, 2048, 640, 1536
        return {
            "x": _w((lambda *s: _rng.normal(s) * 0.05)(B, S, D)),
            "w_gate": _w((lambda *s: _rng.normal(s) * 0.05)(D, F)),
            "w_up": _w((lambda *s: _rng.normal(s) * 0.05)(D, F)),
            "w_down": _w((lambda *s: _rng.normal(s) * 0.05)(F, D)),
        }
    _B_in = _B_setup()

    return {
        "A_x": _A_in["x"],
        "A_w_r": _A_in["w_r"],
        "A_w_i": _A_in["w_i"],
        "B_x": _B_in["x"],
        "B_w_gate": _B_in["w_gate"],
        "B_w_up": _B_in["w_up"],
        "B_w_down": _B_in["w_down"],
    }

def reference(A_x, A_w_r, A_w_i, B_x, B_w_gate, B_w_up, B_w_down):
    def _A_ref(x, w_r, w_i):
        B, S, D = x.shape
        X = (lambda x, axes=(-2,-1): jnp.fft.rfft2(x.astype(jnp.float32), axes=axes))(x, axes=(-2, -1))
        W = w_r + 1j * w_i
        X = X * W
        y = (lambda x, s, axes=(-2,-1): jnp.fft.irfft2(x, s=s, axes=axes).astype(jnp.bfloat16))(X, (S, D), axes=(-2, -1))
        return y

    def _B_ref(x, w_gate, w_up, w_down):
        g = _silu(x @ w_gate)
        u = x @ w_up
        return (g * u) @ w_down

    x = A_x
    xn = _layernorm(x, axis=-1)
    s = _A_ref(xn, A_w_r, A_w_i)
    g = _silu(_B_ref(xn, B_w_gate, B_w_up, B_w_down))
    return x + s * g
```

```python
import numpy as np
import jax
import jax.numpy as jnp
import jax.experimental.pallas as pl
import jax.experimental.pallas.tpu as pltpu

S, D, F, DF = 2048, 640, 1536, 321
TM = 512
NA = S // TM
NT = TM // 128
NC, TG = 6, 256
NB = 6
UB = 2
SB = NB // UB
UC = 2
OCUT = ((0, 2), (2, 4), (4, 5))
ORDER_A = ('dpppgpppppg',) + ('dgppdgpppgpppgppppgppppg',) * 3
ORDER = 'u0u0u0u0u01u1u1u11'
TN = F // NB
R0 = 80
NROW = R0 + 4 * 64
NG = NROW // 8
GB = NG // NB
WN0 = NA * 5 * (TM // 2)
WNS = 64 * 33
P0 = WN0 + 3 * WNS
NW = 22
BF, F32 = jnp.bfloat16, jnp.float32


def _constants():
    b = np.arange(128)
    j = np.arange(32)
    def thb(kd):
        return 2 * np.pi * np.arange(64)[:, None] * kd[None, :] / D
    kd0 = np.concatenate([5 + 10 * j, 10 * np.arange(R0 - 32)])
    f0 = np.concatenate([np.cos(thb(kd0)), -np.sin(thb(kd0))], 1).T * np.tile(kd0 <= 320, 2)[:, None]
    is5 = np.tile(kd0 % 10 == 5, 2)[:, None]
    fs = [np.concatenate([f0 * ~is5, f0 * is5], 1)]
    g0 = np.concatenate([np.cos(thb(kd0[:64])), -np.sin(thb(kd0[:64]))], 1) * (2.0 / D)
    g0[:, 32], g0[:, 96] = 1.0 / D, np.cos(np.pi * np.arange(64)) / D
    is5 = np.tile(kd0[:64] % 10 == 5, 2)[None, :]
    gs = [np.concatenate([g0 * is5, g0 * ~is5], 0)]
    for r in (1, 2, 3, 4):
        th = thb(np.concatenate([r + 10 * j, 10 - r + 10 * j]))
        sg = np.concatenate([np.ones(32), -np.ones(32)])
        c, s = np.cos(th), np.sin(th)
        fsg = sg if r < 3 else -sg
        fs.append(np.block([[c, -s], [fsg * s, fsg * c]]).T)
        gs.append(np.block([[c, -s], [sg * s, sg * c]]) * (2.0 / D))
    ms = []
    for par in (0, 1):
        th = 2 * np.pi * np.outer(b[:64], 2 * b[:64] + par) / 128
        c, s = np.cos(th), np.sin(th)
        ms.append(np.concatenate([np.block([[c, -s], [s, c]]),
                                  np.block([[c.T, s.T], [-s.T, c.T]]) / S], 1))
    th = 2 * np.pi * np.arange(16)[:, None, None] * b[None, None, :] / S
    th = np.broadcast_to(th, (16, 8, 128)).reshape(128, 128)
    tw = np.concatenate([np.cos(th), np.sin(th)], 0).astype(np.float32)
    return np.concatenate([np.pad(f, ((0, 0), (0, 128))) for f in fs + gs] + ms, 0).astype(BF), tw


_CM, _TW = _constants()
_RHO = sum(rho << (4 * (n + 2)) for n, rho in enumerate((1, 6, 4, 9, 2, 7)))
_GROUP = {rho: R0 // 8 + 4 * n for n, rho in enumerate((1, 6, 4, 9, 2, 7, 3, 8))}
_C1, _C2 = float(np.cos(2 * np.pi / 5)), float(np.cos(4 * np.pi / 5))
_S1, _S2 = float(np.sin(2 * np.pi / 5)), float(np.sin(4 * np.pi / 5))


def _rot(z, k, n, sign):
    re, im = z
    k %= n
    if k == 0:
        return re, im
    c, s = float(np.cos(2 * np.pi * k / n)), float(sign * np.sin(2 * np.pi * k / n))
    if (8 * k) % n == 0 and (4 * k) % n:
        a = re - im if c * s > 0 else re + im
        d = re + im if c * s > 0 else im - re
        return a * c, d * c
    return re * c - im * s, re * s + im * c


def _dft4(z, sign):
    (ar, ai), (br, bi), (cr, ci), (dr, di) = z
    pr, pi, qr, qi = ar + cr, ai + ci, ar - cr, ai - ci
    tr, ti, ur, ui = br + dr, bi + di, br - dr, bi - di
    u, v = (qr - ui, qi + ur), (qr + ui, qi - ur)
    if sign < 0:
        u, v = v, u
    return [(pr + tr, pi + ti), u, (pr - tr, pi - ti), v]


def _dft16(z, sign):
    cols = [_dft4([z[4 * a + b] for a in range(4)], sign) for b in range(4)]
    out = [None] * 16
    for k1 in range(4):
        col = []
        for b in range(4):
            re, im = cols[b][k1]
            if (b * k1) == 4:
                col.append((-im, re) if sign > 0 else (im, -re))
            else:
                col.append(_rot((re, im), b * k1, 16, sign))
        for k2, val in enumerate(_dft4(col, sign)):
            out[k1 + 4 * k2] = val
    return out


def _silu(v):
    h = 0.5 * v
    return h + h * jnp.tanh(h)


def _swap(v):
    return pltpu.roll(v, 64, 1)


def _mix(lo, hi):
    lane = jax.lax.broadcasted_iota(jnp.int32, lo.shape, 1)
    return jnp.where(lane < 64, lo, hi)


def _nt(a, b):
    return jax.lax.dot_general(a, b, (((1,), (1,)), ((), ())), preferred_element_type=F32)


def _nn(a, b):
    return jnp.dot(a, b, preferred_element_type=F32)


def _kernel(x_hbm, wr_hbm, wi_hbm, wg_hbm, wu_hbm, wd_hbm, cm_hbm, tw_hbm, o_hbm,
            x_v, fr_v, fi_v, u_v, wg_v, wu_v, wd_v, cm_v, tw_ref, g_v, h_v,
            zr_v, zi_v, yr_v, yi_v, wt_v, o_v, sem, osem):
    step = pl.program_id(0)
    fd_ref, gd_ref, ms_ref = cm_v.at[0:672], cm_v.at[672:1312], cm_v.at[1312:1568]
    cp_x = [None] + [pltpu.make_async_copy(x_hbm.at[TM * c:TM * c + TM], x_v.at[c], sem.at[c])
                     for c in range(1, NA)]
    cp_x0 = [pltpu.make_async_copy(x_hbm.at[TM // 2 * c:TM // 2 * (c + 1)],
                                   x_v.at[0, TM // 2 * c:TM // 2 * (c + 1)], sem.at[NA + NB + NC + 6 + c])
             for c in range(2)]
    cp_u = [pltpu.make_async_copy(wu_hbm.at[:, TN * c:TN * c + TN], wu_v.at[c], sem.at[NA + c])
            for c in range(NB)]
    cp_g = [pltpu.make_async_copy(wg_hbm.at[:, TG * c:TG * c + TG], wg_v.at[c], sem.at[NA + NB + c])
            for c in range(NC)]
    cp_d, cp_c, cp_m, cp_t, cp_r, cp_i = [
        pltpu.make_async_copy(src, dst, sem.at[NA + NB + NC + n_]) for n_, (src, dst) in enumerate(
            ((wd_hbm, wd_v), (cm_hbm.at[0:672], fd_ref),
             (cm_hbm.at[672:1568], cm_v.at[672:1568]), (tw_hbm, tw_ref), (wr_hbm, fr_v), (wi_hbm, fi_v)))]

    pl.when(step == 1 + SB)(lambda: cp_d.wait())

    def cp_o(i, n):
        lanes = slice(128 * OCUT[n][0], 128 * OCUT[n][1])
        return pltpu.make_async_copy(o_v.at[i, :, lanes], o_hbm.at[i, :, lanes], osem.at[i * len(OCUT) + n])

    def dyn(row):
        return row if isinstance(row, int) else pl.multiple_of(jnp.maximum(row, 0), 8)

    def layernorm(c, r0=0, nr=TM):
        words = pltpu.bitcast(x_v[c, r0:r0 + nr, :], jnp.uint32)
        halves = []
        for bits in (words << 16, words & jnp.uint32(0xFFFF0000)):
            x = pltpu.bitcast(bits, F32)
            xc = x - jnp.mean(x, axis=-1, keepdims=True)
            var = jnp.mean(xc * xc, axis=-1, keepdims=True)
            xn = (xc * jax.lax.rsqrt(var + 1e-5)).astype(BF)
            halves.append(pltpu.bitcast(xn.astype(F32), jnp.uint32))
        xn = (halves[0] >> 16) | halves[1]
        for a in range(5):
            u_v[pl.ds(dyn((5 * c + a) * (TM // 2) + r0 // 2), nr // 2), :] = xn[:, 128 * a:128 * a + 128]

    def load_xn(c, r0=0, nr=TM):
        return pltpu.bitcast(jnp.concatenate(
            [u_v[pl.ds((5 * c + a) * (TM // 2) + r0 // 2, nr // 2), :] for a in range(5)], 1), BF)

    def gate(stage, c, r0=0, nr=TM):
        g_v[c, stage, r0:r0 + nr] = _nn(load_xn(stage, r0, nr), wg_v[c]).astype(BF)

    def filter_pass1(t8):
        lanes = slice(128 * t8, 128 * t8 + 128)
        tail = []
        for src in (fr_v, fi_v):
            nyq = pltpu.bitcast(src[320:DF, lanes].astype(F32), jnp.uint32) >> 16
            tail += [pltpu.bitcast(src[256:320, lanes], jnp.uint32),
                     jnp.broadcast_to(nyq, (8, 128)), jnp.zeros((24, 128), jnp.uint32)]
        blocks = [pltpu.bitcast(fr_v[0:256, lanes], jnp.uint32),
                  pltpu.bitcast(fi_v[0:256, lanes], jnp.uint32), jnp.concatenate(tail, 0)]
        for c, blk in enumerate(blocks):
            blk = blk.T
            for q in range(4):
                u_v[pl.ds(WN0 + c * WNS + 33 * (4 * t8 + q), 32), :] = blk[32 * q:32 * q + 32]

    def filter_pass2(k4):
        k1 = k4
        src = wt_v.at[k4 % 8]
        rows = [[u_v[pl.ds(WN0 + c * WNS + 16 * par + k1, 64, stride=33), :] for par in range(2)]
                for c in range(3)]
        for par in range(2):
            src[par, 0:128] = jnp.concatenate([rows[0][par], rows[1][par]], 0).T
        tail = jnp.concatenate(rows[2], 0).T
        tr, ti = tail[0:40], tail[64:104]
        src[2, 0:48] = jnp.concatenate([_mix(tr, _swap(ti)), tail[40:48]], 0)
        src[2, 64:112] = jnp.concatenate([_mix(_swap(tr), ti), tail[40:48]], 0)
        for part in range(2):
            for res in range(5):
                for jj in range(4):
                    j0 = res + 40 * jj
                    if jj < 3:
                        val = src[part, pl.ds(j0, 8, stride=5), :]
                    else:
                        n_lo = (127 - j0) // 5 + 1
                        val = jnp.concatenate(
                            [src[part, pl.ds(j0, n_lo, stride=5), :],
                             src[2, pl.ds(64 * part + j0 + 5 * n_lo - 128, 8 - n_lo, stride=5), :]], 0)
                    u_v[pl.ds(dyn(P0 + (part * NW + 4 * res + jj) * 128 + 8 * k1), 8), :] = val
            for jj in range(4, (R0 - 32) // 8):
                val = src[2, pl.ds(64 * part + 8 * jj, 8), :]
                u_v[pl.ds(dyn(P0 + (part * NW + 16 + jj) * 128 + 8 * k1), 8), :] = val

    def d_forward(stage):
        xf = load_xn(stage).astype(F32)
        x0, x1, x2, x3, x4 = [xf[:, 128 * a:128 * a + 128] for a in range(5)]
        p, q, m, n = x1 + x4, x2 + x3, x1 - x4, x2 - x3
        t0 = x0 + p + q
        t0s = _swap(t0)
        u = {0: _mix(t0 + t0s, t0s - t0).astype(BF)}
        for r, re, im in ((1, x0 + _C1 * p + _C2 * q, -_S1 * m - _S2 * n),
                          (2, x0 + _C2 * p + _C1 * q, _S1 * n - _S2 * m)):
            c, s = float(np.cos(np.pi * r / 5)), float(np.sin(np.pi * r / 5))
            res, ims = _swap(re), _swap(im)
            ev = _mix(re, ims)
            od = c * _mix(res, im) + s * _mix(ims, -re)
            u[r], u[r + 5] = (ev + od).astype(BF), (ev - od).astype(BF)
        yield
        for rho in (0, 1, 6, 2, 7):
            r = min(rho, 10 - rho)
            if rho == 0:
                z, groups = _nt(fd_ref[0:160, 0:128], u[0]), list(range(R0 // 8))
            else:
                z = _nt(fd_ref[32 + 128 * r:160 + 128 * r, 0:128], u[rho])
                groups = [_GROUP[c] + g for c in (r, 10 - r) for g in range(4)]
            for t in range(NT):
                lanes = slice(128 * t, 128 * t + 128)
                for k, g in enumerate(groups):
                    zr_v[g, NT * stage + t] = z[8 * k:8 * k + 8, lanes]
                    zi_v[g, NT * stage + t] = z[8 * (len(groups) + k):8 * (len(groups) + k + 1), lanes]

    def phase_a(stage):
        dfwd = d_forward(stage)
        if stage == 0:
            half = TM // 2
            cp_x0[0].start()
            cp_g[0].start()
            cp_x0[0].wait()
            cp_x0[1].start()
            cp_g[1].start()
            layernorm(0, 0, half)
            cp_g[0].wait()
            cp_g[2].start()
            cp_g[3].start()
            gate(0, 0, 0, half)
            cp_x0[1].wait()
            cp_g[1].wait()
            for cp in cp_g[4:] + [cp_c, cp_x[1]]:
                cp.start()
            gate(0, 1, 0, half)
            layernorm(0, half, half)
            gate(0, 0, half, half)
            gate(0, 1, half, half)
            cp_g[2].wait()
            cp_g[3].wait()
            gate(0, 2)
            next(dfwd)
            gate(0, 3)
            for cp in cp_g[4:] + [cp_c, cp_x[1]]:
                cp.wait()
            for cp in cp_x[2:] + [cp_r, cp_i]:
                cp.start()
        if stage == 1:
            cp_x[2].wait()
            cp_x[3].wait()
            for cp in cp_u + [cp_t, cp_m]:
                cp.start()
        if stage == 2:
            cp_r.wait()
            cp_i.wait()
            cp_d.start()
        chunks, pieces = iter(range(NC - ORDER_A[stage].count('g'), NC)), iter(range(16))
        for item in ORDER_A[stage]:
            if item == 'g':
                gate(stage, next(chunks))
            elif item == 'd':
                next(dfwd, None)
            else:
                n = next(pieces)
                if stage < 2:
                    layernorm(stage + 1 + n // 8, 64 * (n % 8), 64)
                elif stage == 2:
                    filter_pass1(n)
                else:
                    filter_pass2(n)

    @pl.when(step == 0)
    def _():
        for stage in range(NA):
            phase_a(stage)
        for cp in cp_u + [cp_t, cp_m]:
            cp.wait()

    def up_proj(j, rb):
        up = _nn(load_xn(rb), wu_v[j])
        h_v[j, rb] = (_silu(g_v[j, rb].astype(F32)) * up).astype(BF)

    def spectral_b(j):
        base = j * GB
        lhs = []
        for g8 in range(GB):
            if g8 == 4:
                yield
            z = [(zr_v[base + g8, a],
                  zi_v[base + g8, a]) for a in range(16)]
            z = _dft16(z, -1)
            re, im = [z[0][0]], [z[0][1]]
            for k in range(1, 16):
                c, s = tw_ref[8 * k:8 * k + 8, :], tw_ref[128 + 8 * k:136 + 8 * k, :]
                re.append(z[k][0] * c + z[k][1] * s)
                im.append(z[k][1] * c - z[k][0] * s)
            re, im = jnp.concatenate(re, 0), _swap(jnp.concatenate(im, 0))
            lo, hi = _mix(re, im), _swap(_mix(im, re))
            lhs.append(((lo + hi).astype(BF), (lo - hi).astype(BF)))
        f = [_nn(jnp.concatenate([v[par] for v in lhs], 0), ms_ref[128 * par:128 * par + 128, 0:128])
             for par in range(2)]
        yield
        wr, wi = [], []
        for g8 in range(GB):
            g = base + g8
            q = jnp.maximum(g - 2, 0) // 4
            rho = jnp.where(q < 8, (_RHO >> (4 * jnp.minimum(q, 7))) & 15, 5 * q - 37)
            wgrp = jnp.where(g < 10, jnp.where(g < 4, 8 + g, jnp.where(g < 8, g - 4, g + 12)),
                             4 * (rho // 2) + (g - 2) % 4)
            odd = jnp.where(g < 10, (g < 4).astype(jnp.int32), rho % 2)
            shift = (16 * (1 - odd)).astype(jnp.uint32)
            for part, dst in enumerate((wr, wi)):
                word = u_v[pl.ds(dyn(P0 + (part * NW + wgrp) * 128), 128), :]
                dst.append(pltpu.bitcast((word << shift) & jnp.uint32(0xFFFF0000), F32))
        y = []
        for par, w in enumerate((wr, wi)):
            w = jnp.concatenate(w, 0)
            ws = _swap(w)
            prod = f[par] * _mix(w, ws) + _swap(f[par]) * _mix(-ws, w)
            y.append(_nn(prod.astype(BF), ms_ref[128 * par:128 * par + 128, 128:256]))
        yield
        lo, hi = y[0] + y[1], _swap(y[0] - y[1])
        yr, yi = _mix(lo, hi), _swap(_mix(hi, lo))
        for g8 in range(GB):
            if g8 == 4:
                yield
            z = []
            for k in range(16):
                a = yr[g8 * 128 + 8 * k:g8 * 128 + 8 * k + 8]
                b = yi[g8 * 128 + 8 * k:g8 * 128 + 8 * k + 8]
                if k:
                    c, s = tw_ref[8 * k:8 * k + 8, :], tw_ref[128 + 8 * k:136 + 8 * k, :]
                    a, b = a * c - b * s, b * c + a * s
                z.append((a, b))
            for a, (re, im) in enumerate(_dft16(z, 1)):
                yr_v[base + g8, a] = re
                yi_v[base + g8, a] = im

    @pl.when(jnp.logical_and(step >= 1, step < 1 + SB))
    def _phase_b():
        j0 = UB * (step - 1)
        ups = iter([(j0 + n // NA, n % NA) for n in range(UB * NA)])
        specs = [spectral_b(j0 + n) for n in range(UB)]
        for item in ORDER:
            if item == 'u':
                up_proj(*next(ups))
            else:
                next(specs[int(item)], None)

    def phase_c(i):

        def spectrum(*groups):
            rows = []
            for src in (yr_v, yi_v):
                for g in [g0 + k for g0 in groups for k in range(4)]:
                    val = jnp.concatenate([src[g, NT * i + t] for t in range(NT)], 1)
                    if src is yi_v and g == 4:
                        nyq = jnp.concatenate([yr_v[8, NT * i + t] for t in range(NT)], 1)
                        val = jnp.where(jax.lax.broadcasted_iota(jnp.int32, val.shape, 0) == 0, nyq, val)
                    rows.append(val)
            return jnp.concatenate(rows, 0).astype(BF)

        def radix5(v0, v1, v2):
            a1, b1, a2, b2 = v1[:64], v1[64:], v2[:64], v2[64:]
            p, q = v0 + _C1 * a1 + _C2 * a2, v0 + _C2 * a1 + _C1 * a2
            m, n = _S1 * b1 + _S2 * b2, _S2 * b1 - _S1 * b2
            return [v0 + a1 + a2, p - m, q - n, q + n, p + m]

        hid = jnp.concatenate([h_v[c, i] for c in range(NB)], 1)

        def down(n):
            return _nn(hid, wd_v[:, 128 * OCUT[n][0]:128 * OCUT[n][1]])

        ff = [down(0)]
        v05 = _nn(gd_ref[0:128, 0:128], spectrum(0, 4))
        v5, v0 = v05[:64], v05[64:]
        v = [_nn(gd_ref[128 * r:128 * r + 128, 0:128], spectrum(_GROUP[r], _GROUP[10 - r]))
             for r in (1, 2, 3, 4)]
        ff.append(down(1))
        even = radix5(v0, v[1], v[3])
        odd = radix5(v5, jnp.concatenate([v[2][:64], -v[2][64:]], 0),
                     jnp.concatenate([v[0][:64], -v[0][64:]], 0))
        half = [even[a % 5] + odd[a % 5] if a % 2 == 0 else even[a % 5] - odd[a % 5] for a in range(10)]
        cols = [jnp.concatenate(half[2 * t:2 * t + 2], 0) for t in range(5)]
        cols = [c.T for c in cols]
        for n, (t0, t1) in enumerate(OCUT):
            lanes = slice(128 * t0, 128 * t1)
            if n == len(ff):
                ff.append(down(n))
            o_v[i, :, lanes] = (x_v[i, :, lanes].astype(F32)
                                + jnp.concatenate(cols[t0:t1], 1) * _silu(ff[n])).astype(BF)
            cp_o(i, n).start()

    @pl.when(step >= 1 + SB)
    def _():
        for n in range(UC):
            phase_c(UC * jnp.clip(step - (1 + SB), 0, NA // UC - 1) + n)

    @pl.when(step == SB + NA // UC)
    def _():
        for i in range(NA):
            for n in range(len(OCUT)):
                cp_o(i, n).wait()


@jax.jit
def pallas_recurrent_scan__spectral_gfnet__swiglu_ffn__prompt_kernel(
    A_x, A_w_r, A_w_i, B_x, B_w_gate, B_w_up, B_w_down,
):
    del B_x
    hbm = pl.BlockSpec(memory_space=pltpu.HBM)
    out = pl.pallas_call(
        _kernel,
        grid=(1 + SB + NA // UC,),
        in_specs=[hbm] * 8,
        out_specs=hbm,
        out_shape=jax.ShapeDtypeStruct((NA, TM, D), BF),
        scratch_shapes=[
            pltpu.VMEM((NA, TM, D), BF), pltpu.VMEM((DF, S), BF), pltpu.VMEM((DF, S), BF),
            pltpu.VMEM((P0 + 2 * NW * 128, 128), jnp.uint32),
            pltpu.VMEM((NC, D, TG), BF), pltpu.VMEM((NB, D, TN), BF), pltpu.VMEM((F, D), BF),
            pltpu.VMEM(_CM.shape, BF), pltpu.VMEM(_TW.shape, F32),
            pltpu.VMEM((NB, NA, TM, TN), BF), pltpu.VMEM((NB, NA, TM, TN), BF),
            pltpu.VMEM((NG, 16, 8, 128), F32), pltpu.VMEM((NG, 16, 8, 128), F32),
            pltpu.VMEM((NG, 16, 8, 128), F32), pltpu.VMEM((NG, 16, 8, 128), F32),
            pltpu.VMEM((8, 3, 136, 128), jnp.uint32),
            pltpu.VMEM((NA, TM, D), BF),
            pltpu.SemaphoreType.DMA((NA + NB + NC + 8,)),
            pltpu.SemaphoreType.DMA((NA * len(OCUT),)),
        ],
        compiler_params=pltpu.CompilerParams(
            dimension_semantics=("arbitrary",), vmem_limit_bytes=100 * 1024 * 1024,
            flags={'XLA_TPU_EVENLY_DISTRIBUTE_CRITICAL_NODES': True}),
    )(A_x.reshape(S, D), A_w_r.T, A_w_i.T, B_w_gate, B_w_up, B_w_down, _CM, _TW)
    return out.reshape(1, S, D)
```
